```python
import os as _os
_os.environ.setdefault("JAX_PLATFORMS", "cpu")
import jax
import jax.numpy as jnp

def _softmax(x, axis=-1):
    return jax.nn.softmax(x, axis=axis)
def _gelu(x):
    return jax.nn.gelu(x, approximate=True)
def _silu(x):
    return jax.nn.silu(x)
def _sigmoid(x):
    return jax.nn.sigmoid(x)
def _layernorm(x, axis=-1, eps=1e-5):
    m = jnp.mean(x, axis=axis, keepdims=True)
    v = jnp.var(x, axis=axis, keepdims=True)
    return (x - m) / jnp.sqrt(v + eps)
def _scatter_add(tgt, idx, src, axis=0):
    return tgt.at[idx].add(src)
def _segment_sum(src, seg, n):
    return jax.ops.segment_sum(src, seg, n)
class _Rng:
    def __init__(self, key):
        self._k = key
    def _next(self):
        self._k, sub = jax.random.split(self._k)
        return sub
    def normal(self, shape):
        return jax.random.normal(self._next(), shape, dtype=jnp.bfloat16)
    def randint(self, lo, hi, shape):
        return jax.random.randint(self._next(), shape, lo, hi, dtype=jnp.int32)
    def uniform(self, shape, lo=0.0, hi=1.0):
        return jax.random.uniform(self._next(), shape, jnp.bfloat16, lo, hi)
    def permutation(self, n):
        return jax.random.permutation(self._next(), n)


kernel_name = 'standalone__gqa_block_cached__sampling'

def setup_inputs():
    _rng = _Rng(jax.random.key(int.from_bytes(__import__("os").urandom(4), "little")))
    _w = (lambda a: (lambda t: t.astype(jnp.bfloat16) if jnp.issubdtype(t.dtype, jnp.floating) else t)(jnp.asarray(a)))
    B, Sq, D = 32, 16, 1024
    Hq, Hkv, Sk, Dh = 32, 4, 2048, 128
    assert Hq % Hkv == 0, (Hq, Hkv)
    return {
        "x": _w((lambda *s: _rng.normal(s) * 0.8)(B, Sq, D)),
        "k_cache": _w((lambda *s: _rng.normal(s) * 0.8)(B, Hkv, Sk, Dh)),
        "v_cache": _w((lambda *s: _rng.normal(s) * 0.05)(B, Hkv, Sk, Dh)),
        "wq": _w((lambda *s: _rng.normal(s) * 0.8)(D, Hq * Dh) * (D ** -0.5)),
        "wo": _w((lambda *s: _rng.normal(s) * 0.05)(Hq * Dh, D) * ((Hq * Dh) ** -0.5)),
    }

def reference(x, k_cache, v_cache, wq, wo):
    B, Sq, D = x.shape
    Hq, Dh = 32, 128
    Hkv = k_cache.shape[1]
    rep = Hq // Hkv
    q = (lambda x, *d: x.transpose(*d))((x @ wq).reshape(B, Sq, Hq, Dh), 0, 2, 1, 3)
    k = jnp.repeat(k_cache, rep, axis=1)
    v = jnp.repeat(v_cache, rep, axis=1)
    scores = jnp.einsum("bhqd,bhkd->bhqk", q, k) * (Dh ** -0.5)
    p = _softmax(scores, axis=-1)
    o = jnp.einsum("bhqk,bhkd->bhqd", p, v)
    return (lambda x, *d: x.transpose(*d))(o, 0, 2, 1, 3).reshape(B, Sq, Hq * Dh) @ wo
```

```python
import functools

import jax
import jax.numpy as jnp
import jax.experimental.pallas as pl
import jax.experimental.pallas.tpu as pltpu


def _attn_kernel(x_ref, k_ref, v_ref, wq_ref, wo_ref, o_ref, q_scr, a_scr,
                 *, B, Sq, Hq, Hkv, Dh, scale):
    b = pl.program_id(0)
    rep = Hq // Hkv

    @pl.when(b == 0)
    def _():
        x2 = x_ref[...].reshape(B * Sq, x_ref.shape[-1])
        q = jnp.dot(x2, wq_ref[...], preferred_element_type=jnp.float32)
        q_scr[...] = (q * scale).astype(q_scr.dtype).reshape(B, Sq, Hq * Dh)

    qb = q_scr[b]
    outs = []
    for g in range(Hkv):
        qg = jnp.concatenate(
            [qb[:, (g * rep + h) * Dh:(g * rep + h + 1) * Dh] for h in range(rep)],
            axis=0)
        k = k_ref[0, g]
        v = v_ref[0, g]
        s = jax.lax.dot_general(qg, k, (((1,), (1,)), ((), ())),
                                preferred_element_type=jnp.float32)
        m = jnp.max(s, axis=1, keepdims=True)
        p = jnp.exp(s - m)
        l = jnp.sum(p, axis=1, keepdims=True)
        o = jnp.dot(p.astype(v.dtype), v, preferred_element_type=jnp.float32)
        o = o / l
        for h in range(rep):
            outs.append(o[h * Sq:(h + 1) * Sq, :].astype(a_scr.dtype))
    a_scr[b] = jnp.concatenate(outs, axis=1)

    @pl.when(b == B - 1)
    def _():
        a2 = a_scr[...].reshape(B * Sq, Hq * Dh)
        out = jnp.dot(a2, wo_ref[...], preferred_element_type=jnp.float32)
        o_ref[...] = out.astype(o_ref.dtype).reshape(o_ref.shape)


@jax.jit
def pallas_standalone__gqa_block_cached__sampling_kernel(
    x: jax.Array,
    k_cache: jax.Array,
    v_cache: jax.Array,
    wq: jax.Array,
    wo: jax.Array,
):
    B, Sq, D = x.shape
    _, Hkv, Sk, Dh = k_cache.shape
    Hq = wq.shape[1] // Dh
    scale = float(Dh) ** -0.5

    kernel = functools.partial(
        _attn_kernel, B=B, Sq=Sq, Hq=Hq, Hkv=Hkv, Dh=Dh, scale=scale)

    return pl.pallas_call(
        kernel,
        grid=(B,),
        in_specs=[
            pl.BlockSpec((B, Sq, D), lambda b: (0, 0, 0)),
            pl.BlockSpec((1, Hkv, Sk, Dh), lambda b: (b, 0, 0, 0)),
            pl.BlockSpec((1, Hkv, Sk, Dh), lambda b: (b, 0, 0, 0)),
            pl.BlockSpec((D, Hq * Dh), lambda b: (0, 0)),
            pl.BlockSpec((Hq * Dh, D), lambda b: (0, 0)),
        ],
        out_specs=pl.BlockSpec((B, Sq, D), lambda b: (0, 0, 0)),
        out_shape=jax.ShapeDtypeStruct((B, Sq, D), x.dtype),
        scratch_shapes=[
            pltpu.VMEM((B, Sq, Hq * Dh), jnp.bfloat16),
            pltpu.VMEM((B, Sq, Hq * Dh), jnp.bfloat16),
        ],
        compiler_params=pltpu.CompilerParams(
            dimension_semantics=("arbitrary",),
            vmem_limit_bytes=100 * 1024 * 1024,
        ),
    )(x, k_cache, v_cache, wq, wo)
```

```python
import functools

import jax
import jax.numpy as jnp
import jax.experimental.pallas as pl
import jax.experimental.pallas.tpu as pltpu


def _kernel(x_ref, k_hbm, v_hbm, wq_hbm, wo_hbm, o_ref,
            kbuf, vbuf, wqbuf, wobuf, acc, ksem, vsem, wsem,
            *, B, Sq, Hq, Hkv, Dh, scale, bb, nbuf):
    g = pl.program_id(0)
    j = pl.program_id(1)
    nj = B // bb
    nsteps = Hkv * nj
    rep = Hq // Hkv
    t = g * nj + j
    slot = t % nbuf
    G = rep * Dh
    R = bb * Sq

    def k_copy(step, sl, bi):
        gg = step // nj
        jj = step % nj
        return pltpu.make_async_copy(
            k_hbm.at[jj * bb + bi, gg], kbuf.at[sl, bi], ksem.at[sl, bi])

    def v_copy(step, sl, bi):
        gg = step // nj
        jj = step % nj
        return pltpu.make_async_copy(
            v_hbm.at[jj * bb + bi, gg], vbuf.at[sl, bi], vsem.at[sl, bi])

    def wq_copy(gg):
        return pltpu.make_async_copy(
            wq_hbm.at[:, pl.ds(gg * G, G)], wqbuf.at[gg % 2], wsem.at[0, gg % 2])

    def wo_copy(gg):
        return pltpu.make_async_copy(
            wo_hbm.at[pl.ds(gg * G, G), :], wobuf.at[gg % 2], wsem.at[1, gg % 2])

    def start_step(step):
        sl = step % nbuf
        for bi in range(bb):
            k_copy(step, sl, bi).start()
        for bi in range(bb):
            v_copy(step, sl, bi).start()

    @pl.when(t == 0)
    def _():
        wq_copy(0).start()
        start_step(0)
        wo_copy(0).start()
        for s in range(1, nbuf - 1):
            start_step(s)

    @pl.when(t + nbuf - 1 < nsteps)
    def _():
        start_step(t + nbuf - 1)

    @pl.when(jnp.logical_and(j == 0, g + 1 < Hkv))
    def _():
        wq_copy(g + 1).start()
        wo_copy(g + 1).start()

    @pl.when(j == 0)
    def _():
        wq_copy(g).wait()

    rows = pl.ds(pl.multiple_of(j * R, R), R)
    x2 = x_ref[rows, :]
    q = jnp.dot(x2, wqbuf[g % 2], preferred_element_type=jnp.float32)
    q = (q * scale).astype(jnp.bfloat16)

    for bi in range(bb):
        k_copy(t, slot, bi).wait()

    ps, ls = [], []
    for bi in range(bb):
        qb = q[bi * Sq:(bi + 1) * Sq, :]
        qg = jnp.concatenate(
            [qb[:, h * Dh:(h + 1) * Dh] for h in range(rep)], axis=0)
        k = kbuf[slot, bi]
        s = jax.lax.dot_general(qg, k, (((1,), (1,)), ((), ())),
                                preferred_element_type=jnp.float32)
        m = jnp.max(s, axis=1, keepdims=True)
        p = jnp.exp(s - m)
        ls.append(jnp.sum(p, axis=1, keepdims=True))
        ps.append(p.astype(jnp.bfloat16))

    for bi in range(bb):
        v_copy(t, slot, bi).wait()

    outs = []
    for bi in range(bb):
        v = vbuf[slot, bi]
        o = jnp.dot(ps[bi], v, preferred_element_type=jnp.float32)
        o = o / ls[bi]
        outs.append(jnp.concatenate(
            [o[h * Sq:(h + 1) * Sq, :].astype(jnp.bfloat16) for h in range(rep)],
            axis=1))
    a = jnp.concatenate(outs, axis=0)

    @pl.when(j == 0)
    def _():
        wo_copy(g).wait()

    part = jnp.dot(a, wobuf[g % 2], preferred_element_type=jnp.float32)

    @pl.when(g == 0)
    def _():
        acc[rows, :] = part

    @pl.when(jnp.logical_and(g > 0, g < Hkv - 1))
    def _():
        acc[rows, :] += part

    @pl.when(g == Hkv - 1)
    def _():
        o_ref[rows, :] = (acc[rows, :] + part).astype(o_ref.dtype)


@jax.jit
def pallas_standalone__gqa_block_cached__sampling_kernel(
    x: jax.Array,
    k_cache: jax.Array,
    v_cache: jax.Array,
    wq: jax.Array,
    wo: jax.Array,
):
    B, Sq, D = x.shape
    _, Hkv, Sk, Dh = k_cache.shape
    Hq = wq.shape[1] // Dh
    rep = Hq // Hkv
    scale = float(Dh) ** -0.5
    bb = 4 if B % 4 == 0 else (2 if B % 2 == 0 else 1)
    nbuf = 2
    G = rep * Dh
    assert Hkv >= 2

    kernel = functools.partial(
        _kernel, B=B, Sq=Sq, Hq=Hq, Hkv=Hkv, Dh=Dh, scale=scale, bb=bb, nbuf=nbuf)

    out = pl.pallas_call(
        kernel,
        grid=(Hkv, B // bb),
        in_specs=[
            pl.BlockSpec((B * Sq, D), lambda g, j: (0, 0)),
            pl.BlockSpec(memory_space=pl.ANY),
            pl.BlockSpec(memory_space=pl.ANY),
            pl.BlockSpec(memory_space=pl.ANY),
            pl.BlockSpec(memory_space=pl.ANY),
        ],
        out_specs=pl.BlockSpec((B * Sq, D), lambda g, j: (0, 0)),
        out_shape=jax.ShapeDtypeStruct((B * Sq, D), x.dtype),
        scratch_shapes=[
            pltpu.VMEM((nbuf, bb, Sk, Dh), jnp.bfloat16),
            pltpu.VMEM((nbuf, bb, Sk, Dh), jnp.bfloat16),
            pltpu.VMEM((2, D, G), jnp.bfloat16),
            pltpu.VMEM((2, G, D), jnp.bfloat16),
            pltpu.VMEM((B * Sq, D), jnp.float32),
            pltpu.SemaphoreType.DMA((nbuf, bb)),
            pltpu.SemaphoreType.DMA((nbuf, bb)),
            pltpu.SemaphoreType.DMA((2, 2)),
        ],
        compiler_params=pltpu.CompilerParams(
            dimension_semantics=("arbitrary", "arbitrary"),
            vmem_limit_bytes=64 * 1024 * 1024,
        ),
    )(x.reshape(B * Sq, D), k_cache, v_cache, wq, wo)
    return out.reshape(B, Sq, D)
```
